```python
import os as _os
_os.environ.setdefault("JAX_PLATFORMS", "cpu")
import jax
import jax.numpy as jnp

def _softmax(x, axis=-1):
    return jax.nn.softmax(x, axis=axis)
def _gelu(x):
    return jax.nn.gelu(x, approximate=True)
def _silu(x):
    return jax.nn.silu(x)
def _sigmoid(x):
    return jax.nn.sigmoid(x)
def _layernorm(x, axis=-1, eps=1e-5):
    m = jnp.mean(x, axis=axis, keepdims=True)
    v = jnp.var(x, axis=axis, keepdims=True)
    return (x - m) / jnp.sqrt(v + eps)
def _scatter_add(tgt, idx, src, axis=0):
    return tgt.at[idx].add(src)
def _segment_sum(src, seg, n):
    return jax.ops.segment_sum(src, seg, n)
class _Rng:
    def __init__(self, key):
        self._k = key
    def _next(self):
        self._k, sub = jax.random.split(self._k)
        return sub
    def normal(self, shape):
        return jax.random.normal(self._next(), shape, dtype=jnp.bfloat16)
    def randint(self, lo, hi, shape):
        return jax.random.randint(self._next(), shape, lo, hi, dtype=jnp.int32)
    def uniform(self, shape, lo=0.0, hi=1.0):
        return jax.random.uniform(self._next(), shape, jnp.bfloat16, lo, hi)
    def permutation(self, n):
        return jax.random.permutation(self._next(), n)


kernel_name = 'parallel_sum__sliding_local_dilated__glu_gated_geglu__prompt'

def setup_inputs():
    _rng = _Rng(jax.random.key(int.from_bytes(__import__("os").urandom(4), "little")))
    _w = (lambda a: (lambda t: t.astype(jnp.bfloat16) if jnp.issubdtype(t.dtype, jnp.floating) else t)(jnp.asarray(a)))
    def _A_setup():
        B, S, D = 1, 2048, 512
        return {
            "x": _w((lambda *s: _rng.normal(s) * 0.05)(B, S, D)),
            "wqkv": _w((lambda *s: _rng.normal(s) * 0.05)(D, 3 * D)),
            "wo": _w((lambda *s: _rng.normal(s) * 0.05)(D, D)),
        }
    _A_in = _A_setup()

    def _B_setup():
        B, S, Dm, Df = 1, 2048, 512, 1376
        return {
            "x": _w((lambda *s: _rng.normal(s) * 0.05)(B, S, Dm)),
            "w_gate": _w((lambda *s: _rng.normal(s) * 0.1)(Dm, Df) * (Dm ** -0.5)),
            "w_up": _w((lambda *s: _rng.normal(s) * 0.1)(Dm, Df) * (Dm ** -0.5)),
            "w_down": _w((lambda *s: _rng.normal(s) * 0.1)(Df, Dm) * (Df ** -0.5)),
        }
    _B_in = _B_setup()

    return {
        "A_x": _A_in["x"],
        "A_wqkv": _A_in["wqkv"],
        "A_wo": _A_in["wo"],
        "B_x": _B_in["x"],
        "B_w_gate": _B_in["w_gate"],
        "B_w_up": _B_in["w_up"],
        "B_w_down": _B_in["w_down"],
    }

def reference(A_x, A_wqkv, A_wo, B_x, B_w_gate, B_w_up, B_w_down):
    def _A_ref(x, wqkv, wo):
        B, S, D = x.shape
        H = 32; Dh = D // H
        W, dil = 8, 2
        qkv = (lambda x, *d: x.transpose(*d))((x @ wqkv).reshape(B, S, 3, H, Dh), 2, 0, 3, 1, 4)
        q, k, v = qkv[0], qkv[1], qkv[2]
        scale = Dh ** -0.5
        pos = jnp.arange(S)
        off = jnp.arange(W) * dil
        idx = pos[:, None] - off[None, :]
        mask = idx >= 0
        idx_c = jnp.where(mask, idx, 0).reshape(-1)
        kg = k[:, :, idx_c, :].reshape(B, H, S, W, Dh)
        vg = v[:, :, idx_c, :].reshape(B, H, S, W, Dh)
        logits = jnp.einsum("bhsd,bhswd->bhsw", q, kg) * scale
        logits = jnp.where(mask[None, None, :, :], logits, -1e9)
        attn = _softmax(logits, axis=-1)
        o = jnp.einsum("bhsw,bhswd->bhsd", attn, vg)
        return (lambda x, *d: x.transpose(*d))(o, 0, 2, 1, 3).reshape(B, S, D) @ wo

    def _B_ref(x, w_gate, w_up, w_down):
        g = jnp.einsum("bsd,df->bsf", x, w_gate)
        u = jnp.einsum("bsd,df->bsf", x, w_up)
        h = _gelu(g) * u
        return jnp.einsum("bsf,fd->bsd", h, w_down)

    x = A_x
    xn = _layernorm(x, axis=-1)
    return x + _A_ref(xn, A_wqkv, A_wo) + _B_ref(xn, B_w_gate, B_w_up, B_w_down)
```

```python
import functools
import jax
import jax.numpy as jnp
import jax.experimental.pallas as pl
import jax.experimental.pallas.tpu as pltpu

S, D, H, DH, W, DIL, DF = 2048, 512, 32, 16, 8, 2, 1376
T = 256
HALO = 16


def _kernel(x_ref, wqkv_hbm, wo_hbm, wg_hbm, wu_hbm, wd_hbm, o_ref,
            kv_scr, wqkv_raw, wqkv_ref, wo_raw, wo_f32, wo_ref, wg_ref, wu_ref, wd_ref, sems):
    i = pl.program_id(0)

    @pl.when(i == 0)
    def _():
        copies = [
            pltpu.make_async_copy(wqkv_hbm, wqkv_raw, sems.at[0]),
            pltpu.make_async_copy(wg_hbm, wg_ref, sems.at[1]),
            pltpu.make_async_copy(wu_hbm, wu_ref, sems.at[2]),
            pltpu.make_async_copy(wd_hbm, wd_ref, sems.at[3]),
            pltpu.make_async_copy(wo_hbm, wo_raw, sems.at[4]),
        ]
        for c in copies:
            c.start()
        r = jax.lax.broadcasted_iota(jnp.int32, (D, D), 0)
        c_ = jax.lax.broadcasted_iota(jnp.int32, (D, D), 1)
        tgt = (r % DH) * H + r // DH
        perm = jnp.where(c_ == tgt, 1.0, 0.0).astype(jnp.bfloat16)
        copies[0].wait()
        for p in range(3):
            wqkv_ref[:, p * D:(p + 1) * D] = jnp.dot(
                wqkv_raw[:, p * D:(p + 1) * D], perm,
                preferred_element_type=jnp.float32).astype(jnp.bfloat16)
        for c in copies[1:]:
            c.wait()
        for j in range(4):
            wo_f32[j] = wo_raw[:, 128 * j:128 * (j + 1)].astype(jnp.float32)
        for d in range(DH):
            for j in range(4):
                wo_ref[d * H:(d + 1) * H, 128 * j:128 * (j + 1)] = (
                    wo_f32[j, pl.ds(d, H, stride=DH), :].astype(jnp.bfloat16))
        kv_scr[0:HALO, :] = jnp.zeros((HALO, 2 * D), jnp.float32)

    @pl.when(i > 0)
    def _():
        kv_scr[0:HALO, :] = kv_scr[T:T + HALO, :]

    x = x_ref[...].astype(jnp.float32)
    m = jnp.mean(x, axis=-1, keepdims=True)
    xc = x - m
    var = jnp.mean(xc * xc, axis=-1, keepdims=True)
    xn = (xc * jax.lax.rsqrt(var + 1e-5)).astype(jnp.bfloat16)

    qkv = jnp.dot(xn, wqkv_ref[...], preferred_element_type=jnp.float32)
    q = qkv[:, :D] * (DH ** -0.5)
    kv_scr[HALO:, :] = qkv[:, D:]

    row = i * T + jax.lax.broadcasted_iota(jnp.int32, (T, 128), 0)
    logits = []
    for w in range(W):
        kw = kv_scr[pl.ds(HALO - DIL * w, T), 0:D]
        p = q * kw
        s4 = p[:, 0:128] + p[:, 128:256] + p[:, 256:384] + p[:, 384:512]
        s4 = s4 + pltpu.roll(s4, 64, 1)
        s4 = s4 + pltpu.roll(s4, 32, 1)
        if w > 0:
            s4 = jnp.where(row >= DIL * w, s4, -1e9)
        logits.append(s4)
    mx = logits[0]
    for w in range(1, W):
        mx = jnp.maximum(mx, logits[w])
    ps = [jnp.exp(l - mx) for l in logits]
    den = ps[0]
    for w in range(1, W):
        den = den + ps[w]
    inv = 1.0 / den
    acc = [None] * 4
    for w in range(W):
        vw = kv_scr[pl.ds(HALO - DIL * w, T), D:2 * D]
        for j in range(4):
            t = ps[w] * vw[:, 128 * j:128 * (j + 1)]
            acc[j] = t if acc[j] is None else acc[j] + t
    o = jnp.concatenate([a * inv for a in acc], axis=1).astype(jnp.bfloat16)
    a_out = jnp.dot(o, wo_ref[...], preferred_element_type=jnp.float32)

    nt = (((1,), (1,)), ((), ()))
    g = jax.lax.dot_general(xn, wg_ref[...], nt, preferred_element_type=jnp.float32)
    u = jax.lax.dot_general(xn, wu_ref[...], nt, preferred_element_type=jnp.float32)
    h = (jax.nn.gelu(g, approximate=True) * u).astype(jnp.bfloat16)
    b_out = jnp.dot(h, wd_ref[...], preferred_element_type=jnp.float32)
    o_ref[...] = (x + a_out + b_out).astype(o_ref.dtype)


@jax.jit
def pallas_parallel_sum__sliding_local_dilated__glu_gated_geglu__prompt_kernel(
    A_x, A_wqkv, A_wo, B_x, B_w_gate, B_w_up, B_w_down,
):
    x = A_x.reshape(S, D)
    anyspec = pl.BlockSpec(memory_space=pltpu.MemorySpace.HBM)
    out = pl.pallas_call(
        _kernel,
        grid=(S // T,),
        in_specs=[
            pl.BlockSpec((T, D), lambda i: (i, 0)),
            anyspec, anyspec, anyspec, anyspec, anyspec,
        ],
        out_specs=pl.BlockSpec((T, D), lambda i: (i, 0)),
        out_shape=jax.ShapeDtypeStruct((S, D), jnp.bfloat16),
        scratch_shapes=[
            pltpu.VMEM((T + HALO, 2 * D), jnp.float32),
            pltpu.VMEM((D, 3 * D), jnp.bfloat16),
            pltpu.VMEM((D, 3 * D), jnp.bfloat16),
            pltpu.VMEM((D, D), jnp.bfloat16),
            pltpu.VMEM((4, D, 128), jnp.float32),
            pltpu.VMEM((D, D), jnp.bfloat16),
            pltpu.VMEM((DF, D), jnp.bfloat16),
            pltpu.VMEM((DF, D), jnp.bfloat16),
            pltpu.VMEM((DF, D), jnp.bfloat16),
            pltpu.SemaphoreType.DMA((5,)),
        ],
        compiler_params=pltpu.CompilerParams(
            dimension_semantics=("arbitrary",),
            vmem_limit_bytes=96 * 1024 * 1024,
        ),
    )(x, A_wqkv, A_wo, B_w_gate.T, B_w_up.T, B_w_down)
    return out.reshape(1, S, D)
```

```python
import functools

import jax
import jax.numpy as jnp
import jax.experimental.pallas as pl
import jax.experimental.pallas.tpu as pltpu

S, D, H, DH, W, DIL, DF = 2048, 512, 32, 16, 8, 2, 1376
T = 256
C = 32
GC = 128
RH = 128
HALO = 16
NT = S // T
NG = (DF + GC - 1) // GC
NA = T // C
NR = T // RH
_NT_DIMS = (((1,), (1,)), ((), ()))


def _layernorm_bf16(x_bf16):
    x = x_bf16.astype(jnp.float32)
    m = jnp.mean(x, axis=-1, keepdims=True)
    xc = x - m
    var = jnp.mean(xc * xc, axis=-1, keepdims=True)
    return (xc * jax.lax.rsqrt(var + 1e-5)).astype(jnp.bfloat16)


def _attn_chunk(first, c, qkv_scr, o_scr):
    r0 = c * C
    logits = [None] * W
    for ph in range(4):
        base = HALO + r0 - 8 - DIL * ph
        for j in range(4):
            qj = qkv_scr[pl.ds(HALO + r0, C), 128 * j:128 * (j + 1)]
            kj = qkv_scr[pl.ds(base, C + 8), D + 128 * j:D + 128 * (j + 1)]
            a = qj * kj[8:]
            b = qj * kj[:C]
            logits[ph] = a if logits[ph] is None else logits[ph] + a
            logits[ph + 4] = b if logits[ph + 4] is None else logits[ph + 4] + b
    for w in range(W):
        s4 = logits[w]
        s4 = s4 + pltpu.roll(s4, 64, 1)
        s4 = s4 + pltpu.roll(s4, 32, 1)
        if first and w > 0 and r0 < DIL * w:
            row = r0 + jax.lax.broadcasted_iota(jnp.int32, (C, 128), 0)
            s4 = jnp.where(row >= DIL * w, s4, -1e9)
        logits[w] = s4
    mx = logits[0]
    for w in range(1, W):
        mx = jnp.maximum(mx, logits[w])
    ps = [jnp.exp(l - mx) for l in logits]
    den = ps[0]
    for w in range(1, W):
        den = den + ps[w]
    inv = 1.0 / den
    for j in range(4):
        acc = None
        for ph in range(4):
            base = HALO + r0 - 8 - DIL * ph
            vj = qkv_scr[pl.ds(base, C + 8), 2 * D + 128 * j:2 * D + 128 * (j + 1)]
            t = ps[ph] * vj[8:] + ps[ph + 4] * vj[:C]
            acc = t if acc is None else acc + t
        o_scr[pl.ds(r0, C), 128 * j:128 * (j + 1)] = (acc * inv).astype(jnp.bfloat16)


def _kernel(x_hbm, wqkv_hbm, wo_hbm, wg_hbm, wu_hbm, wd_hbm, o_ref,
            x_all, xn_scr, qkv_scr, o_scr, h_scr, wqkv_raw, wqkv_ref, wo_raw, t_scr, wo_ref,
            wg_ref, wu_ref, wd_ref, sems):
    i = pl.program_id(0)

    def qkv_rows(xn, rr):
        qkv_scr[HALO + rr * RH:HALO + (rr + 1) * RH, :] = jax.lax.dot_general(
            xn[rr * RH:(rr + 1) * RH], wqkv_ref[...], _NT_DIMS,
            preferred_element_type=jnp.float32)

    def x_tile(t):
        if isinstance(t, int):
            return x_all[t * T:(t + 1) * T, :]
        return x_all[pl.ds(pl.multiple_of(t * T, T), T), :]

    def body(first, last):
        t = 0 if first else i
        if first:
            qkv_copies = [
                pltpu.make_async_copy(wqkv_hbm.at[:, p * D:(p + 1) * D],
                                      wqkv_raw.at[:, p * D:(p + 1) * D], sems.at[p])
                for p in range(3)]
            ga = [pltpu.make_async_copy(wg_hbm, wg_ref, sems.at[3]),
                  pltpu.make_async_copy(wu_hbm, wu_ref, sems.at[4])]
            gc_ = [pltpu.make_async_copy(wd_hbm, wd_ref, sems.at[5]),
                   pltpu.make_async_copy(wo_hbm, wo_raw, sems.at[6]),
                   pltpu.make_async_copy(x_hbm.at[T:2 * T], x_all.at[T:2 * T], sems.at[7])]
            x0_copy = pltpu.make_async_copy(x_hbm.at[:T], x_all.at[:T], sems.at[8])
            xr_copy = pltpu.make_async_copy(x_hbm.at[2 * T:], x_all.at[2 * T:], sems.at[9])
            qkv_copies[0].start()
            x0_copy.start()
            for c in qkv_copies[1:]:
                c.start()
            for p in range(3):
                qkv_copies[p].wait()
                if p == 1:
                    x0_copy.wait()
                    for c in ga:
                        c.start()
                    xn = _layernorm_bf16(x_tile(0))
                for j in range(4):
                    blk = wqkv_raw[128 * j:128 * (j + 1), p * D:(p + 1) * D].astype(jnp.float32)
                    if p == 0:
                        blk = blk * (DH ** -0.5)
                    t_scr[j] = blk.T
                for d in range(DH):
                    for j in range(4):
                        wqkv_ref[p * D + d * H:p * D + (d + 1) * H, 128 * j:128 * (j + 1)] = (
                            t_scr[j, pl.ds(d, H, stride=DH), :].astype(jnp.bfloat16))
            qkv_scr[0:HALO, D:] = jnp.zeros((HALO, 2 * D), jnp.float32)
            for rr in range(NR):
                qkv_rows(xn, rr)
            for ca in range(NA):
                _attn_chunk(first, ca, qkv_scr, o_scr)
            for cp in ga:
                cp.wait()
            for c in gc_:
                c.start()
        else:
            xn = xn_scr[...]

        for c in range(NG):
            if not first:
                for rr in range(1, NR):
                    if c == (rr * NG) // NR:
                        qkv_rows(xn, rr)
            lo = c * GC
            hi = min(DF, lo + GC)
            g = jax.lax.dot_general(xn, wg_ref[lo:hi, :], _NT_DIMS,
                                    preferred_element_type=jnp.float32)
            u = jax.lax.dot_general(xn, wu_ref[lo:hi, :], _NT_DIMS,
                                    preferred_element_type=jnp.float32)
            h_scr[:, lo:hi] = (jax.nn.gelu(g, approximate=True) * u).astype(jnp.bfloat16)
        if not first:
            for c in range(NA):
                _attn_chunk(first, c, qkv_scr, o_scr)

        if first:
            for cp in gc_:
                cp.wait()
            xr_copy.start()
            for j in range(4):
                t_scr[j] = wo_raw[:, 128 * j:128 * (j + 1)].astype(jnp.float32)
            for d in range(DH):
                for j in range(4):
                    wo_ref[d * H:(d + 1) * H, 128 * j:128 * (j + 1)] = (
                        t_scr[j, pl.ds(d, H, stride=DH), :].astype(jnp.bfloat16))
        if first or last:
            b_out = jnp.dot(h_scr[...], wd_ref[...], preferred_element_type=jnp.float32)
            a_out = jnp.dot(o_scr[...], wo_ref[...], preferred_element_type=jnp.float32)
        else:
            a_out = jnp.dot(o_scr[...], wo_ref[...], preferred_element_type=jnp.float32)
            b_out = jnp.dot(h_scr[...], wd_ref[...], preferred_element_type=jnp.float32)
        o_ref[...] = (x_tile(t).astype(jnp.float32) + a_out + b_out).astype(o_ref.dtype)

        if not last:
            xn2 = _layernorm_bf16(x_tile(t + 1))
            xn_scr[...] = xn2
            qkv_scr[0:HALO, D:] = qkv_scr[T:T + HALO, D:]
            qkv_rows(xn2, 0)
        if first:
            xr_copy.wait()

    pl.when(i == 0)(functools.partial(body, True, False))
    pl.when(jnp.logical_and(i > 0, i < NT - 1))(functools.partial(body, False, False))
    pl.when(i == NT - 1)(functools.partial(body, False, True))


@jax.jit
def pallas_parallel_sum__sliding_local_dilated__glu_gated_geglu__prompt_kernel(
    A_x: jax.Array,
    A_wqkv: jax.Array,
    A_wo: jax.Array,
    B_x: jax.Array,
    B_w_gate: jax.Array,
    B_w_up: jax.Array,
    B_w_down: jax.Array,
):
    del B_x
    x = A_x.reshape(S, D)
    hbm = pl.BlockSpec(memory_space=pltpu.MemorySpace.HBM)
    out = pl.pallas_call(
        _kernel,
        grid=(NT,),
        in_specs=[hbm, hbm, hbm, hbm, hbm, hbm],
        out_specs=pl.BlockSpec((T, D), lambda i: (i, 0)),
        out_shape=jax.ShapeDtypeStruct((S, D), jnp.bfloat16),
        scratch_shapes=[
            pltpu.VMEM((S, D), jnp.bfloat16),
            pltpu.VMEM((T, D), jnp.bfloat16),
            pltpu.VMEM((T + HALO, 3 * D), jnp.float32),
            pltpu.VMEM((T, D), jnp.bfloat16),
            pltpu.VMEM((T, DF), jnp.bfloat16),
            pltpu.VMEM((D, 3 * D), jnp.bfloat16),
            pltpu.VMEM((3 * D, D), jnp.bfloat16),
            pltpu.VMEM((D, D), jnp.bfloat16),
            pltpu.VMEM((4, D, 128), jnp.float32),
            pltpu.VMEM((D, D), jnp.bfloat16),
            pltpu.VMEM((DF, D), jnp.bfloat16),
            pltpu.VMEM((DF, D), jnp.bfloat16),
            pltpu.VMEM((DF, D), jnp.bfloat16),
            pltpu.SemaphoreType.DMA((10,)),
        ],
        compiler_params=pltpu.CompilerParams(
            dimension_semantics=("arbitrary",),
            vmem_limit_bytes=96 * 1024 * 1024,
        ),
    )(x, A_wqkv, A_wo, B_w_gate.T, B_w_up.T, B_w_down)
    return out.reshape(1, S, D)
```
